```python
import os as _os
_os.environ.setdefault('JAX_PLATFORMS', 'cpu')
import jax
import jax.numpy as jnp

def _softmax(x, axis=-1):
    return jax.nn.softmax(x, axis=axis)

def _gelu(x):
    return jax.nn.gelu(x, approximate=True)

def _silu(x):
    return jax.nn.silu(x)

def _sigmoid(x):
    return jax.nn.sigmoid(x)

def _layernorm(x, axis=-1, eps=1e-05):
    m = jnp.mean(x, axis=axis, keepdims=True)
    v = jnp.var(x, axis=axis, keepdims=True)
    return (x - m) / jnp.sqrt(v + eps)

def _scatter_add(tgt, idx, src, axis=0):
    return tgt.at[idx].add(src)

def _segment_sum(src, seg, n):
    return jax.ops.segment_sum(src, seg, n)

class _Rng:

    def __init__(self, key):
        self._k = key

    def _next(self):
        self._k, sub = jax.random.split(self._k)
        return sub

    def normal(self, shape):
        return jax.random.normal(self._next(), shape, dtype=jnp.bfloat16)

    def randint(self, lo, hi, shape):
        return jax.random.randint(self._next(), shape, lo, hi, dtype=jnp.int32)

    def uniform(self, shape, lo=0.0, hi=1.0):
        return jax.random.uniform(self._next(), shape, jnp.bfloat16, lo, hi)

    def permutation(self, n):
        return jax.random.permutation(self._next(), n)
kernel_name = 'adaLN_cond__sliding_local_dilated__mixer_channel_mlp__prompt'

def setup_inputs():
    _rng = _Rng(jax.random.key(int.from_bytes(__import__("os").urandom(4), "little")))
    _w = lambda a: (lambda t: t.astype(jnp.bfloat16) if jnp.issubdtype(t.dtype, jnp.floating) else t)(jnp.asarray(a))

    def _A_setup():
        B, S, D = (1, 2048, 512)
        return {'x': _w((lambda *s: _rng.normal(s) * 0.05)(B, S, D)), 'wqkv': _w((lambda *s: _rng.normal(s) * 0.05)(D, 3 * D)), 'wo': _w((lambda *s: _rng.normal(s) * 0.05)(D, D))}
    _A_in = _A_setup()

    def _B_setup():
        B, S, D, F = (1, 2048, 512, 1792)
        return {'x': _w((lambda *s: _rng.normal(s) * 0.05)(B, S, D)), 'w1': _w((lambda *s: _rng.normal(s) * 0.8)(D, F) * D ** (-0.5)), 'b1': _w((lambda *s: _rng.normal(s) * 0.8)(F)), 'w2': _w((lambda *s: _rng.normal(s) * 0.8)(F, D) * F ** (-0.5)), 'b2': _w((lambda *s: _rng.normal(s) * 0.4)(D))}
    _B_in = _B_setup()
    return {'A_x': _A_in['x'], 'A_wqkv': _A_in['wqkv'], 'A_wo': _A_in['wo'], 'B_x': _B_in['x'], 'B_w1': _B_in['w1'], 'B_b1': _B_in['b1'], 'B_w2': _B_in['w2'], 'B_b2': _B_in['b2'], 'c': _w((lambda *s: _rng.normal(s) * 0.05)(1, 512) * 8.0), 'w_mod': _w((lambda *s: _rng.normal(s) * 0.05)(512, 6 * 512) * 512 ** (-0.5) * 8.0)}

def reference(A_x, A_wqkv, A_wo, B_x, B_w1, B_b1, B_w2, B_b2, c, w_mod):

    def _A_ref(x, wqkv, wo):
        B, S, D = x.shape
        H = 32
        Dh = D // H
        W, dil = (8, 2)
        qkv = (lambda x, *d: x.transpose(*d))((x @ wqkv).reshape(B, S, 3, H, Dh), 2, 0, 3, 1, 4)
        q, k, v = (qkv[0], qkv[1], qkv[2])
        scale = Dh ** (-0.5)
        pos = jnp.arange(S)
        off = jnp.arange(W) * dil
        idx = pos[:, None] - off[None, :]
        mask = idx >= 0
        idx_c = jnp.where(mask, idx, 0).reshape(-1)
        kg = k[:, :, idx_c, :].reshape(B, H, S, W, Dh)
        vg = v[:, :, idx_c, :].reshape(B, H, S, W, Dh)
        logits = jnp.einsum('bhsd,bhswd->bhsw', q, kg) * scale
        logits = jnp.where(mask[None, None, :, :], logits, -1000000000.0)
        attn = _softmax(logits, axis=-1)
        o = jnp.einsum('bhsw,bhswd->bhsd', attn, vg)
        return (lambda x, *d: x.transpose(*d))(o, 0, 2, 1, 3).reshape(B, S, D) @ wo

    def _B_ref(x, w1, b1, w2, b2):
        y = _layernorm(x, axis=-1)
        h = _gelu(jnp.einsum('bsd,df->bsf', y, w1) + b1)
        return jnp.einsum('bsf,fd->bsd', h, w2) + b2
    x = A_x
    mod = (_silu(c) @ w_mod).reshape(c.shape[0], 6, 1, -1)
    sa, ca, ga, sb, cb, gb = (mod[:, 0].copy(), mod[:, 1].copy(), mod[:, 2].copy(), mod[:, 3].copy(), mod[:, 4].copy(), mod[:, 5].copy())
    h = _layernorm(x, axis=-1) * (1 + ca) + sa
    x = x + ga * _A_ref(h, A_wqkv, A_wo)
    h = _layernorm(x, axis=-1) * (1 + cb) + sb
    x = x + gb * _B_ref(h, B_w1, B_b1, B_w2, B_b2)
    return x
```

```python
import functools
import math

import jax
import jax.numpy as jnp
from jax import lax
import jax.experimental.pallas as pl
import jax.experimental.pallas.tpu as pltpu

S, D, DH, W, DIL, F = 2048, 512, 16, 8, 2, 1792
L = 128
NC = D // L
NF = F // L // 2
HALO = 16
T = 256
U = 32
G = 8
NT, NU, TH = S // T, T // U, T // 2
EPS = 1e-5
LOG2E = math.log2(math.e)
GA = (math.sqrt(2.0 / math.pi) * 0.044715) ** (1.0 / 3.0)
GC = math.sqrt(2.0 / math.pi) / GA
f32, bf16, u32 = jnp.float32, jnp.bfloat16, jnp.uint32

PLAN = dict(t1=0, ep=2, ta=1, sk=2, so=0, eo=0, rel=40, laga=5, lagl=9, lagh=8, lagp=5, gapl=5, gaph=8,
            h0=0, h1=34, z1=6, b0=71, b1=4, b2=14, b3=7, b4=9, b5=11, b6=6, b7=10, o0=0, o1=76, m1=64,
            p0=21, p1=120, p2=21, p3=104, a1=0, ao=9, a2=18, s1=0, e1=10, l0=4, l1=38, s2=0, e2=10, k1=20,
            v0=34, v1=48, x0=2, x1=4, y0=52, y1=74)
LOCAL = {
    'q1': dict(lagp=8, gaph=4),
    'q2': dict(rel=72, lagp=10),
    'q3': dict(laga=4, rel=32),
    'q4': dict(laga=7, gaph=6),
    'q5': dict(h1=30, gaph=6, rel=56),
    'q6': dict(laga=7, gaph=6, h1=36),
    'q7': dict(laga=4, lagp=2),
    '0': dict(l1=39, rel=56, e1=4, ao=5, a1=2, e2=8, lagp=7, s1=10),
    '1': dict(l1=36, e2=14, e1=12, so=2, t1=3),
    '2': dict(l1=35, lagl=7, s1=10, rel=56, e1=6, a1=2, eo=2, laga=6),
    '3': dict(s1=5, e2=12, l1=36, a1=1, rel=48, l0=6, laga=4, gapl=9, eo=2, lagl=11),
    '4': dict(s1=5, e2=12, rel=48, lagl=11, a2=20),
    '5': dict(rel=56, e1=8, ta=2, gapl=3),
    '6': dict(rel=72, a2=17),
}


def _dot(a, b):
    return jnp.dot(a, b, preferred_element_type=f32)


def _put(ref, p, rows, cols, v):
    ref[pl.ds(p, 1), rows, cols] = v[None].astype(bf16)


def _mean(v):
    return jnp.sum(v, axis=-1, keepdims=True) * (1.0 / D)


def _lhs7(a11, a12, a21, a22):
    return (a11 + a22, a21 + a22, a11, a22, a11 + a12, a21 - a11, a12 - a22)


def _rhs7(b11, b12, b21, b22):
    return (b11 + b22, b11, b12 - b22, b21 - b11, b22, b11 + b12, b21 + b22)


def _strassen(prod, emit, bias=None):
    m5 = prod(4)
    yield
    m3 = prod(2)
    if bias is not None:
        m3 = m3 + bias[1]
    emit(0, 1, m3 + m5)
    yield
    m2 = prod(1)
    t22 = m3 - m2
    yield
    m4 = prod(3)
    if bias is not None:
        m4 = m4 + bias[0]
    emit(1, 0, m2 + m4)
    t11 = m4 - m5
    yield
    m1 = prod(0)
    t11 = t11 + m1
    t22 = t22 + m1
    yield
    emit(0, 0, t11 + prod(6))
    yield
    emit(1, 1, t22 + prod(5))
    yield


def _staged(n, stages, skew=1, split=False):
    state = {}
    for t in range(n + skew * (len(stages) - 1)):
        for s in reversed(range(len(stages))):
            u = t - skew * s
            if 0 <= u < n:
                state[u] = stages[s](u, state.get(u))
                if split:
                    yield
        if not split:
            yield


def _run(gen):
    for _ in gen:
        pass


def _head_major(chunks):
    lane = lax.broadcasted_iota(jnp.int32, chunks[0].shape, 1)
    out = []
    for jp in range(NC):
        y = chunks[0]
        for j in range(1, NC):
            y = jnp.where(((lane >> 2) & 3) == ((j + jp) & 3), chunks[j], y)
        src = 16 * (lane & 7) + 4 * ((((lane >> 3) & 3) + jp) & 3) + (lane >> 5)
        out.append(jnp.take_along_axis(y, src, axis=1))
    return out


def _kernel(x_hbm, wqkv_hbm, wo_hbm, w1_hbm, b1_hbm, w2_hbm, b2_hbm, c_hbm, wmod_hbm, o_hbm,
            x_v, wqkv_v, wo_v, w1_v, w2_v, wmod_v, c_v, b1_v, b2_v,
            wqkv_s, wo_s, w1_s, w2_s, y_s, q_s, k_s, v_s, wof_s, t_s, m_s, o_v,
            sems, osems, h_s, a_s, g_s, x1_s):
    loads = []

    def load_async(src, dst):
        i = len(loads)
        loads.append(lambda z=0: pltpu.make_async_copy(src, dst, sems.at[i + z]))
        loads[-1]().start()
        return loads[-1]

    def cols(src, dst, a, n):
        return load_async(src.at[:, pl.ds(a, n)], dst.at[:, pl.ds(a, n)])

    def tiles(a, b):
        return load_async(x_hbm.at[0, pl.ds(a * T, (b - a) * T)], x_v.at[pl.ds(a * T, (b - a) * T)])

    cols0 = ((0, 2 * L), (2 * L, 2 * L), (D, 2 * L), (D + 2 * L, L), (D + 3 * L, L))
    cp_c, cp_q, cp_x0 = load_async(c_hbm, c_v), cols(wqkv_hbm, wqkv_v, 0, D), tiles(0, 1)
    cp_m0 = [cols(wmod_hbm, wmod_v, a, n) for a, n in cols0]
    cp_x1, cp_k, cp_v = tiles(1, 2), cols(wqkv_hbm, wqkv_v, D, D), cols(wqkv_hbm, wqkv_v, 2 * D, D)
    cp_x2, cp_x3, cp_x5 = tiles(2, 3), tiles(3, 5), tiles(5, NT)
    cp_wo, cp_w1 = load_async(wo_hbm, wo_v), load_async(w1_hbm, w1_v)
    cp_m1 = cols(wmod_hbm, wmod_v, 2 * D, 4 * D)
    cp_w2, cp_b1, cp_b2 = load_async(w2_hbm, w2_v), load_async(b1_hbm, b1_v), load_async(b2_hbm, b2_v)

    def pin(i, carry):
        for r in (wqkv_s, wo_s, w1_s, w2_s, q_s):
            r[i, pl.ds(0, 8), pl.ds(0, L)] = jnp.zeros((8, L), r.dtype)
        m_s[pl.ds(pl.multiple_of(i * 8, 8), 8), pl.ds(0, L)] = jnp.zeros((8, L), f32)
        return i - 1

    zero = lax.fori_loop(0, 2, pin, 0)
    dyn = lambda r0: pl.multiple_of(zero * 16 + r0, 16)
    wqkv_s, wo_s, w1_s, w2_s, y_s = (r.bitcast(bf16) for r in (wqkv_s, wo_s, w1_s, w2_s, y_s))
    h_s, a_s, g_s = ([r.bitcast(bf16) for r in rs] for rs in (h_s, a_s, g_s))

    never = lax.broadcasted_iota(jnp.int32, (8, L), 0) < zero
    tie = dict(last=None, due=[], now=0, lagp=0)
    past = []

    def after_mxu(v, lead):
        old = [u for t, u in past if t <= tie['now'] - lead]
        return jnp.where(never, old[-1], v) if old else v

    def before_mxu(v, lag, gap=0):
        for r in range(0, v.shape[0], 8):
            tie['due'].append((tie['now'] + lag + gap * r / 8, v[r:r + 8, -L:]))

    def mm(a, b, cost=1):
        slots = [(r, c) for c in range(0, a.shape[1], D) for r in range(0, a.shape[0], 16)]
        due, later = {}, []
        for t, v in tie['due']:
            k = int(max(t - tie['now'], 0) / cost * len(slots))
            if k < len(slots):
                due.setdefault(slots[k], []).append(v)
            else:
                later.append((t, v))
        tie['due'] = later

        def tile(r, c):
            v = a[r:r + 16, c:c + L]
            if (r, c) not in due:
                return v
            return pltpu.bitcast(
                jnp.where(never, functools.reduce(jnp.maximum, due[r, c]), pltpu.bitcast(v, f32)), bf16)

        if due:
            a = jnp.concatenate([jnp.concatenate([tile(r, c) for c in range(0, a.shape[1], L)], axis=1)
                                 for r in range(0, a.shape[0], 16)], axis=0)
        out = _dot(a, b)
        past.append((tie['now'], out[:8, :L]))
        return out

    def wait(*copies):
        last = past[-1][1] if past else tie['last']
        z = 0 if last is None else jnp.where(never, pltpu.bitcast(last, jnp.int32), 0)[0, 0]
        for copy in copies:
            copy(z).wait()
        yield

    def combine(dst, p0, r0, n, *quad):
        ops = _rhs7(*quad)
        for p, b in enumerate(ops):
            _put(dst, p0 + p, pl.ds(r0, 16), pl.ds(n * L, L), b)
        if dst is wqkv_s or (r0 // 16 + n) % tie['ep'] == 0:
            before_mxu(ops[0][8:], tie['lagp'])

    def prep_qkv(t):
        def gather(u, _):
            return [_head_major([pltpu.bitcast(wqkv_v[pl.ds(u * 32 + o, 32), pl.ds(t * D + j * L, L)], u32)
                                 for j in range(NC)]) for o in (0, D // 2)]

        def finish(u, st):
            for n in range(2):
                b = [pltpu.bitcast(st[r][n + m], bf16).astype(f32) for r in (0, 1) for m in (0, 2)]
                for r in (0, 16):
                    combine(wqkv_s, t * 7, u * 32 + r, n, *(v[r:r + 16] for v in b))

        return _staged(D // 64, (gather, finish)), D // 64 + 1

    def prep_wo():
        for j in range(NC):
            wof_s[j] = wo_v[:, pl.ds(j * L, L)].astype(f32)
            yield

        def rows(jp, ch, r0):
            return jnp.concatenate(
                [wof_s[ch, pl.ds(L * j + 4 * ((j + jp) & 3) + r // 32, 8, stride=16), :]
                 for r in (r0, r0 + 8) for j in (r // 8 % NC,)], axis=0)

        for k in range(2):
            for r0 in range(0, L, 16):
                for n in range(2):
                    combine(wo_s, 0, k * L + r0, n, *(rows(k + a, n + b, r0) for a in (0, 2) for b in (0, 2)))
                yield

    def prep_w1():
        for j in range(NF):
            for r0 in range(0, D // 2, 32):
                for r in (r0, r0 + 16):
                    lo, hi = (w1_v[pl.ds(r + o, 16), pl.ds(2 * j * L, 2 * L)].astype(f32) for o in (0, D // 2))
                    combine(w1_s, 0, r, j, lo[:, :L], lo[:, L:], hi[:, :L], hi[:, L:])
                yield

    def prep_w2():
        for j in range(NF):
            for r0 in range(0, L, 16):
                b = [w2_v[pl.ds((2 * j + o) * L + r0, 16), pl.ds(m * L, 2 * L)].astype(f32)
                     for o in (0, 1) for m in (0, 2)]
                for n in range(2):
                    combine(w2_s, 0, j * L + r0, n, *(v[:, n * L:(n + 1) * L] for v in b))
                yield

    def modulation(a, n):
        v = _dot(sc, wmod_v[:, pl.ds(a, n)])[:8]
        i = a // D
        m_s[pl.ds(8 * i, 8), pl.ds(a % D, n)] = v + 1.0 if i in (1, 4) else v * (0.5 / GA) if i == 5 else v
        return v[:, -L:]

    def mod(i):
        return jnp.concatenate([m_s[pl.ds(8 * i, 8), :]] * (U // 8), axis=0)

    def put_lhs(dst, u, val, at=dyn):
        for k in range(2):
            lo, hi = val[:, k * L:(k + 1) * L], val[:, (k + 2) * L:(k + 3) * L]
            for p, a in enumerate(_lhs7(lo[:U // 2], hi[:U // 2], lo[U // 2:], hi[U // 2:])):
                _put(dst, p, pl.ds(at(u * U // 2), U // 2), pl.ds(k * L, L), a)

    def center(u, st):
        xc = st[0] - st[1]
        return xc, _mean(xc * xc)

    def ln1(i, last, skew):
        def load(u, _):
            x = x_v[pl.ds(i * T + u * U, U), :].astype(f32)
            return x, _mean(x)

        return _staged(NU, (load, center, lambda u, st: last(u, st[0] * lax.rsqrt(st[1] + EPS))), skew)

    def norm1(i):
        def finish(u, n):
            h = n * mod(1) + mod(0)
            before_mxu(h, tie['lagh'], tie['gaph'] / 10)
            put_lhs(h_s[i % 3], u, h)

        return ln1(i, finish, 2), NU + 4

    def norm2(i, skew=2):
        def load(u, _):
            x1 = x1_s[i % 2][pl.ds(u * U, U), :]
            return x1, _mean(x1)

        def modulate(u, st):
            h = st[0] * lax.rsqrt(st[1] + EPS) * mod(4) + mod(3)
            return h, _mean(h)

        def center2(u, st):
            xc = st[0] - st[1]
            return xc, jnp.sum(xc * xc, axis=-1, keepdims=True) * (1.0 / (D * GA * GA))

        def finish(u, st):
            y = st[0] * lax.rsqrt(st[1] + EPS / (GA * GA))
            before_mxu(y, tie['lagl'], tie['gapl'] / 10)
            put_lhs(y_s, u, y)

        return _staged(NU, (load, center, modulate, center2, finish), skew, True), 5 * NU

    def gemm(src, w, p0, n, emit, cost=1, bias=None):
        return _strassen(lambda p: mm(src[p, pl.ds(0, TH), :], w[p0 + p, :, pl.ds(n * L, L)], cost), emit, bias)

    def gemm_d(src, w, p0, emit, cost=1, bias=None):
        for n in range(2):
            def units(rh, ch, val):
                for u in range(NU):
                    emit(u * U + rh * U // 2, n + 2 * ch, val[u * U // 2:(u + 1) * U // 2])

            yield from gemm(src, w, p0, n, units, cost, bias and (bias[n], bias[n + 2]))

    def qkv(i, t):
        def emit(r, j, val):
            dst = (q_s, k_s, v_s)[t]
            dst[j, pl.ds(HALO + i * T + r, U // 2), :] = val
            if i == 0 and r == 0 and t:
                dst[j, pl.ds(0, HALO), :] = jnp.broadcast_to(val[:1], (HALO, L))

        return gemm_d(h_s[i % 3], wqkv_s, t * 7, emit)

    def attention():
        def logits(g, _):
            scale = after_mxu(jnp.full((G, L), DH ** -0.5 * LOG2E, f32), tie['rel'])
            q = [q_s[j, pl.ds(HALO + g * G, G), :] * scale for j in range(NC)]
            part = [functools.reduce(jnp.add, [q[j] * k_s[j, pl.ds(HALO + g * G - DIL * w, G), :]
                                               for j in range(NC)]) for w in range(W)]
            if tie['t1']:
                before_mxu(part[-1], tie['laga'] + tie['t1'] - 10)
            return [(a, pltpu.roll(a, 64, 1)) for a in part]

        def fold(g, st):
            return [(a, pltpu.roll(a, 32, 1)) for a in (a + b for a, b in st)]

        def mix(g, st):
            lg = [a + b for a, b in st]
            for w in range(W):
                if g * G < DIL * w:
                    pos = g * G + lax.broadcasted_iota(jnp.int32, (G, L), 0)
                    lg[w] = jnp.where(pos >= DIL * w, lg[w], -1e9 * LOG2E)
            m = functools.reduce(jnp.maximum, lg)
            e = [jnp.exp2(t - m) for t in lg]
            den = functools.reduce(jnp.add, e)
            r = pl.reciprocal(den, approx=True)
            r = r * (2.0 - den * r)
            out = [None] * NC
            for w in range(W):
                for j in range(NC):
                    t = e[w] * v_s[j, pl.ds(HALO + g * G - DIL * w, G), :]
                    out[j] = t if out[j] is None else out[j] + t
            unit.append(jnp.concatenate([o * r for o in out], axis=1))
            before_mxu((unit[-1], r, den)[tie['ta']], tie['laga'])
            if len(unit) * G == U:
                put_lhs(a_s[g * G // T % len(a_s)], g * G % T // U, jnp.concatenate(unit, axis=0))
                del unit[:]

        unit = []
        return _staged(S // G, (logits, fold, mix))

    def proj(i):
        def emit(r, j, val):
            c = pl.ds(j * L, L)
            gate = jnp.concatenate([m_s[pl.ds(16, 8), c]] * (U // 16), axis=0)
            x1_s[i % 2][pl.ds(dyn(r), U // 2), c] = x_v[pl.ds(i * T + r, U // 2), c].astype(f32) + gate * val

        return gemm_d(a_s[i % len(a_s)], wo_s, 0, emit)

    def mlp1(i):
        b1 = b1_v[...].astype(f32) * GA
        for j in range(NF):
            g = {}

            def emit(rh, ch, u):
                g[rh, ch] = u + u * jnp.tanh(u * (u * u + GC))
                if len(g) == 4:
                    for p, a in enumerate(_lhs7(g[0, 0], g[0, 1], g[1, 0], g[1, 1])):
                        _put(g_s[i % 2], p, pl.ds(dyn(0), TH), pl.ds(j * L, L), a)

            yield from gemm(y_s, w1_s, 0, j, emit, bias=(b1[2 * j:2 * j + 1], b1[2 * j + 1:2 * j + 2]))

    def mlp2(i):
        b2 = b2_v[...].astype(f32) * (2 * GA)

        def emit(r, j, val):
            c = pl.ds(j * L, L)
            gate = jnp.concatenate([m_s[pl.ds(40, 8), c]] * (U // 16), axis=0)
            o_v[pl.ds(i * T + r, U // 2), c] = (x1_s[i % 2][pl.ds(r, U // 2), c] + gate * val).astype(bf16)

        yield from gemm_d(g_s[i % 2], w2_s, 0, emit, NF / 2, [b2[j:j + 1] for j in range(NC)])

    def out_copy(i):
        k = i - (NT - 1)
        idx = (pl.ds(i * T, T), slice(None)) if k < 0 else (pl.ds(S - T, T), pl.ds(k * L, L))
        return pltpu.make_async_copy(o_v.at[idx], o_hbm.at[(0, *idx)], osems.at[i])

    def store(*parts):
        for i in parts:
            out_copy(i).start()
        yield

    _run(wait(cp_c))
    cf = c_v[...].astype(f32)
    sc = jnp.broadcast_to(cf * jax.nn.sigmoid(cf), (16, D)).astype(bf16)

    def settle():
        tie.update(last=functools.reduce(jnp.maximum, [v for _, v in tie['due']]), due=[])

    def park(u, n):
        t_s[pl.ds(u * U, U), :] = n
        before_mxu(n, 0)

    _run(wait(cp_q))
    _run(prep_qkv(0)[0])
    settle()
    _run(wait(cp_x0))
    _run(ln1(0, park, 3))
    settle()
    for copy, part in zip(cp_m0, cols0):
        _run(wait(copy))
        tie['last'] = modulation(*part)
    for u in range(NU):
        put_lhs(h_s[0], u, t_s[pl.ds(u * U, U), :] * mod(1) + mod(0), int)

    plan, clock = [], [0.0]

    def mxu(gen, n, cost=1):
        t0 = clock[0]
        for _ in range(n):
            plan.append((clock[0], 1, gen))
            clock[0] += cost
        return t0

    def at(t, gen, order=0):
        plan.append((t, order, gen))

    def spread(gen, n, t0, t1):
        plan.extend((t0 + (t1 - t0) * (k + 0.5) / n, 2, gen) for k in range(n))

    def knobs(t, name):
        def apply():
            for k in ('t1', 'ep', 'ta', 'rel', 'laga', 'lagl', 'lagh', 'lagp', 'gapl', 'gaph'):
                tie[k] = knob(k)
            yield

        knob = lambda k: LOCAL.get(str(name), {}).get(k, PLAN[k])
        at(t, apply(), -1)
        return knob

    att, att_steps = attention(), [0]

    def attend(n, t0, t1, tiles_done=0):
        n = min(max(n, tiles_done and tiles_done * T // G + 2 - att_steps[0]), S // G + 2 - att_steps[0])
        att_steps[0] += n
        spread(att, n, t0, t1)

    knobs(0, 'q1')
    for t in range(3):
        mxu(qkv(0, t), 14)
        mxu(qkv(1, t), 14)
    at(PLAN['x0'], wait(cp_x1))
    spread(*norm1(1), PLAN['x0'], PLAN['x1'])
    at(14, wait(cp_k))
    spread(*prep_qkv(1), 14, PLAN['k1'])
    at(PLAN['v0'], wait(cp_v))
    spread(*prep_qkv(2), PLAN['v0'], PLAN['v1'])
    at(PLAN['y0'], wait(cp_x2))
    spread(*norm1(2), PLAN['y0'], PLAN['y1'])
    attend(PLAN['b1'], PLAN['b0'], 84)
    for i in range(2, NT):
        t, last = clock[0], i == NT - 1
        knob = knobs(t, f'q{i}')
        if i == 2:
            at(t, wait(cp_x3))
        if i == 3:
            at(t, wait(cp_x5, cp_wo))
            spread(prep_wo(), NC + 16, t + PLAN['o0'], t + PLAN['o1'])
            at(t + PLAN['p0'], wait(cp_w1))
            spread(prep_w1(), 8 * NF, t + PLAN['p0'], t + PLAN['p1'])
        if i == 5:
            at(t + 7, wait(cp_m1))
            spread((modulation(a, L) for a in range(2 * D, 6 * D, L)), 4 * NC, t + 8, t + 8 + PLAN['m1'])
        if i == 6:
            at(t + PLAN['p2'], wait(cp_w2, cp_b1, cp_b2))
            spread(prep_w2(), 8 * NF, t + PLAN['p2'], t + PLAN['p3'])
        mxu(qkv(i, 0), 14)
        if last:
            tp = mxu(proj(0), 14)
        mxu(qkv(i, 1), 14)
        mxu(qkv(i, 2), 14)
        if last:
            spread(*norm2(0), tp + 15, clock[0] - PLAN['z1'])
        else:
            spread(*norm1(i + 1), t + knob('h0'), t + knob('h1'))
        attend(PLAN[f'b{i}'], t + knob('so'), clock[0] - knob('eo'), i == NT - 2)
    for i in range(NT - 1):
        knob = knobs(clock[0], i)
        t = mxu(mlp1(i), 7 * NF)
        attend(knob('a1'), t + knob('s1'), clock[0] - knob('e1'), i + 2)
        t = mxu(proj(i + 1), 14)
        attend(knob('ao'), t + knob('so'), clock[0] - knob('eo'))
        w2 = mlp2(i)
        keep = i == NT - 2
        t = mxu(w2, 14 - keep, NF / 2)
        spread(*norm2(i + 1, knob('sk')), t + knob('l0'), t + knob('l1') - keep * NF / 2)
        attend(knob('a2'), t + knob('s2'), clock[0] - knob('e2'))
        if not keep:
            at(clock[0], store(i))
    i = NT - 1
    mxu(mlp1(i), 7 * NF)
    mxu(w2, 1, NF / 2)
    at(clock[0], store(i - 1))
    t = mxu(mlp2(i), 14, NF / 2)
    at(t + 7 * NF / 2, store(i, i + 2))
    at(t + 13 * NF / 2, store(i + 1))
    at(clock[0], store(i + 3))
    for tie['now'], _, gen in sorted(plan, key=lambda e: e[:2]):
        next(gen)
    for i in range(NT - 1 + NC):
        out_copy(i).wait()


@jax.jit
def pallas_adaLN_cond__sliding_local_dilated__mixer_channel_mlp__prompt_kernel(
    A_x, A_wqkv, A_wo, B_x, B_w1, B_b1, B_w2, B_b2, c, w_mod,
):
    del B_x
    hbm = pl.BlockSpec(memory_space=pl.ANY)
    lhs = pltpu.VMEM((7, TH // 2 + 8, D // 2), u32)
    return pl.pallas_call(
        _kernel,
        out_shape=jax.ShapeDtypeStruct(A_x.shape, bf16),
        in_specs=[hbm] * 9,
        out_specs=hbm,
        scratch_shapes=[
            pltpu.VMEM((S, D), bf16),
            pltpu.VMEM((D, 3 * D), bf16),
            pltpu.VMEM((D, D), bf16),
            pltpu.VMEM((D, F), bf16),
            pltpu.VMEM((F, D), bf16),
            pltpu.VMEM((D, 6 * D), bf16),
            pltpu.VMEM((1, D), bf16),
            pltpu.VMEM((F // L, L), bf16),
            pltpu.VMEM((NC, L), bf16),
            pltpu.VMEM((3 * 7, D // 4, D // 2), u32),
            pltpu.VMEM((7, D // 4, D // 2), u32),
            pltpu.VMEM((7, D // 4, F // 2), u32),
            pltpu.VMEM((7, F // 4, D // 2), u32),
            lhs,
            *[pltpu.VMEM((NC, HALO + S + 24, L), f32)] * 3,
            pltpu.VMEM((NC, D, L), f32),
            pltpu.VMEM((T, D), f32),
            pltpu.VMEM((48, D), f32),
            pltpu.VMEM((S, D), bf16),
            pltpu.SemaphoreType.DMA((20,)),
            pltpu.SemaphoreType.DMA((NT - 1 + NC,)),
            [lhs] * 3,
            [lhs] * 4,
            [pltpu.VMEM((7, TH // 2, F // 2), u32)] * 2,
            [pltpu.VMEM((T, D), f32)] * 2,
        ],
        compiler_params=pltpu.CompilerParams(
            vmem_limit_bytes=100 * 1024 * 1024, flags={'XLA_TPU_RESCHEDULE_DMA_DONES': True}),
    )(A_x, A_wqkv, A_wo, B_w1, B_b1.reshape(F // L, L), B_w2, B_b2.reshape(NC, L), c, w_mod)
```
